```python
import jax
import jax.numpy as jnp

def _softmax(x, axis=-1):
    return jax.nn.softmax(x, axis=axis)

def _gelu(x):
    return jax.nn.gelu(x, approximate=True)

def _silu(x):
    return jax.nn.silu(x)

def _sigmoid(x):
    return jax.nn.sigmoid(x)

def _layernorm(x, axis=-1, eps=1e-05):
    m = jnp.mean(x, axis=axis, keepdims=True)
    v = jnp.var(x, axis=axis, keepdims=True)
    return (x - m) / jnp.sqrt(v + eps)

def _scatter_add(tgt, idx, src, axis=0):
    return tgt.at[idx].add(src)

def _segment_sum(src, seg, n):
    return jax.ops.segment_sum(src, seg, n)

class _Rng:

    def __init__(self, key):
        self._k = key

    def _next(self):
        self._k, sub = jax.random.split(self._k)
        return sub

    def normal(self, shape):
        return jax.random.normal(self._next(), shape, dtype=jnp.bfloat16)

    def randint(self, lo, hi, shape):
        return jax.random.randint(self._next(), shape, lo, hi, dtype=jnp.int32)

    def uniform(self, shape, lo=0.0, hi=1.0):
        return jax.random.uniform(self._next(), shape, jnp.bfloat16, lo, hi)

    def permutation(self, n):
        return jax.random.permutation(self._next(), n)
kernel_name = 'interleave_layers__linear_kernel_hedgehog__mixer_gmlp__prompt'

def _fwd_setup_inputs():
    _rng = _Rng(jax.random.key(int.from_bytes(__import__("os").urandom(4), "little")))
    _w = lambda a: (lambda t: t.astype(jnp.bfloat16) if jnp.issubdtype(t.dtype, jnp.floating) else t)(jnp.asarray(a))

    def _A_setup():
        B, S, D, H = (1, 2048, 640, 32)
        Dh = D // H
        return {'x': _w((lambda *s: _rng.normal(s) * 0.05)(B, S, D)), 'wqkv': _w((lambda *s: _rng.normal(s) * 0.05)(D, 3 * D)), 'w_phi': _w((lambda *s: _rng.normal(s) * 0.05)(H, Dh, Dh) * Dh ** (-0.5)), 'wo': _w((lambda *s: _rng.normal(s) * 0.05)(D, D))}
    _A_in = _A_setup()

    def _B_setup():
        B, S, D, F = (1, 2048, 640, 1536)
        Fh = F // 2
        return {'x': _w((lambda *s: _rng.normal(s) * 0.05)(B, S, D)), 'w_in': _w((lambda *s: _rng.normal(s) * 0.05)(D, 2 * Fh)), 'w_sp': _w(0.01 * (lambda *s: _rng.normal(s) * 0.05)(S, S)), 'b_sp': _w(1.0 + 0.01 * (lambda *s: _rng.normal(s) * 0.05)(S)), 'w_out': _w((lambda *s: _rng.normal(s) * 0.05)(Fh, D))}
    _B_in = _B_setup()
    return {'A_x': _A_in['x'], 'A_wqkv': _A_in['wqkv'], 'A_w_phi': _A_in['w_phi'], 'A_wo': _A_in['wo'], 'B_x': _B_in['x'], 'B_w_in': _B_in['w_in'], 'B_w_sp': _B_in['w_sp'], 'B_b_sp': _B_in['b_sp'], 'B_w_out': _B_in['w_out']}

def _fwd_reference(A_x, A_wqkv, A_w_phi, A_wo, B_x, B_w_in, B_w_sp, B_b_sp, B_w_out):

    def _A_ref(x, wqkv, w_phi, wo):
        B, S, D = x.shape
        H = 32
        Dh = D // H
        qkv = (lambda x, *d: x.transpose(*d))((x @ wqkv).reshape(B, S, 3, H, Dh), 2, 0, 3, 1, 4)
        q, k, v = (qkv[0], qkv[1], qkv[2])
        pq = jnp.einsum('bhsd,hdf->bhsf', q, w_phi)
        pk = jnp.einsum('bhsd,hdf->bhsf', k, w_phi)
        phi_q = jnp.concatenate([_softmax(pq, axis=-1), _softmax(-pq, axis=-1)], axis=-1)
        phi_k = jnp.concatenate([_softmax(pk, axis=-1), _softmax(-pk, axis=-1)], axis=-1)
        kv = jnp.einsum('bhsf,bhsd->bhfd', phi_k, v)
        z = jnp.einsum('bhsf->bhf', phi_k)
        num = jnp.einsum('bhqf,bhfd->bhqd', phi_q, kv)
        den = jnp.einsum('bhqf,bhf->bhq', phi_q, z)[..., None] + 1e-06
        o = num / den
        return (lambda x, *d: x.transpose(*d))(o, 0, 2, 1, 3).reshape(B, S, D) @ wo

    def _B_ref(x, w_in, w_sp, b_sp, w_out):
        B, S, D = x.shape
        F = w_in.shape[-1]
        Fh = F // 2
        z = _gelu(jnp.einsum('bsd,df->bsf', x, w_in))
        z1 = z[..., :Fh].copy()
        z2 = _layernorm(z[..., Fh:], axis=-1)
        g = jnp.einsum('ts,bsf->btf', w_sp, z2) + b_sp[None, :, None]
        return jnp.einsum('bsf,fd->bsd', z1 * g, w_out)
    x = A_x
    x = x + _A_ref(_layernorm(x, axis=-1), A_wqkv, A_w_phi, A_wo)
    x = x + _B_ref(_layernorm(x, axis=-1), B_w_in, B_w_sp, B_b_sp, B_w_out)
    x = x + _A_ref(_layernorm(x, axis=-1), A_wqkv, A_w_phi, A_wo)
    x = x + _B_ref(_layernorm(x, axis=-1), B_w_in, B_w_sp, B_b_sp, B_w_out)
    return x

def setup_inputs():
    _inp = _fwd_setup_inputs()
    _gk = jax.random.fold_in(jax.random.key(int.from_bytes(__import__("os").urandom(4), "little")), 2 ** 31 - 1)
    _shapes = [[1, 2048, 640]]
    _dtypes = ['bfloat16']
    _gks = jax.random.split(_gk, len(_shapes))
    _gs = [jax.random.normal(k, s, dtype=jnp.dtype(d)) * 0.05 for k, s, d in zip(_gks, _shapes, _dtypes)]
    _inp['grad_out'] = _gs[0]
    return _inp

def reference(A_x, A_wqkv, A_w_phi, A_wo, B_w_in, B_w_sp, B_b_sp, B_w_out, B_x, grad_out):
    _const = dict(B_x=B_x)

    def _f(*_d):
        return _fwd_reference(**{'A_x': _d[0], 'A_wqkv': _d[1], 'A_w_phi': _d[2], 'A_wo': _d[3], 'B_w_in': _d[4], 'B_w_sp': _d[5], 'B_b_sp': _d[6], 'B_w_out': _d[7], **_const})
    _out, _vjp = jax.vjp(_f, A_x, A_wqkv, A_w_phi, A_wo, B_w_in, B_w_sp, B_b_sp, B_w_out)
    _grads = _vjp(grad_out)
    _out0 = jnp.asarray(_out)
    return (_out0, *[jnp.asarray(_g) for _g in _grads])
```

```python
import jax
import jax.numpy as jnp
from jax import lax
import jax.experimental.pallas as pl
import jax.experimental.pallas.tpu as pltpu

S = 2048
D = 640
H = 32
DH = 20
NG = 4
HG = 8
GV = DH * HG
GP = 2 * GV
F = 1536
FH = 768
T = 512
NT = S // T
NL = T // 128
EPS = 1e-5
GELU_C = 0.7978845608028654
GELU_A = 0.044715

f32 = jnp.float32
bf16 = jnp.bfloat16

_NT = (((1,), (1,)), ((), ()))
_TN = (((0,), (0,)), ((), ()))


def _nn(a, b):
    return jnp.dot(a, b, preferred_element_type=f32)


def _nt(a, b):
    return lax.dot_general(a, b, _NT, preferred_element_type=f32)


def _tn(a, b):
    return lax.dot_general(a, b, _TN, preferred_element_type=f32)


def _iota(shape, dim):
    return lax.broadcasted_iota(jnp.int32, shape, dim)


def _eye(n):
    return jnp.where(_iota((n, n), 0) == _iota((n, n), 1), 1.0, 0.0).astype(bf16)


def _ln_fwd(x):
    mu = jnp.mean(x, axis=0, keepdims=True)
    xc = x - mu
    var = jnp.mean(xc * xc, axis=0, keepdims=True)
    rstd = lax.rsqrt(var + EPS)
    return xc * rstd, rstd


def _ln_bwd(dxn, xn, rstd):
    m1 = jnp.mean(dxn, axis=0, keepdims=True)
    m2 = jnp.mean(dxn * xn, axis=0, keepdims=True)
    return rstd * (dxn - m1 - xn * m2)


def _gelu(u):
    t = jnp.tanh(GELU_C * (u + GELU_A * (u * u * u)))
    return 0.5 * u * (1.0 + t)


def _gelu_and_grad(u):
    u2 = u * u
    t = jnp.tanh(GELU_C * (u + GELU_A * (u2 * u)))
    hp = 0.5 * (1.0 + t)
    g = u * hp
    dg = hp + (0.5 * GELU_C) * u * (1.0 - t * t) * (1.0 + (3.0 * GELU_A) * u2)
    return g, dg


def _gelu_grad(u):
    return _gelu_and_grad(u)[1]


def _phi_fwd(p):
    p4 = p.reshape(NG, DH, HG, T)
    mx = jnp.max(p4, axis=1, keepdims=True)
    mn = jnp.min(p4, axis=1, keepdims=True)
    ep = jnp.exp(p4 - mx)
    em = jnp.exp(mn - p4)
    rp = 1.0 / jnp.sum(ep, axis=1, keepdims=True)
    rm = 1.0 / jnp.sum(em, axis=1, keepdims=True)
    ph = jnp.concatenate([ep * rp, em * rm], axis=1)
    return ph.reshape(2 * D, T)


def _phi_bwd(ph, dph):
    ph4 = ph.reshape(NG, 2 * DH, HG, T)
    dph4 = dph.reshape(NG, 2 * DH, HG, T)
    php, phm = ph4[:, :DH], ph4[:, DH:]
    tp = php * dph4[:, :DH]
    tm = phm * dph4[:, DH:]
    sp = jnp.sum(tp, axis=1, keepdims=True)
    sm = jnp.sum(tm, axis=1, keepdims=True)
    dp = (tp - php * sp) - (tm - phm * sm)
    return dp.reshape(D, T)


def _fold(a):
    r = a[:, 0:128]
    for i in range(1, NL):
        r = r + a[:, i * 128:(i + 1) * 128]
    return r


def _tile_lanes(a):
    return jnp.concatenate([a] * NL, axis=1)


def _split_hi_lo(a):
    hi = a.astype(bf16)
    lo = (a - hi.astype(f32)).astype(bf16)
    return hi, lo


def _kernel(
    x_hbm, gout_hbm, wqkv_hbm, wphi_ref, wo_hbm, win_hbm, wsp_hbm, bsp_ref, wout_hbm,
    out_hbm, gx_hbm, dwqkv_hbm, dwphi_ref, dwo_hbm, dwin_hbm, dwsp_hbm, dbsp_ref, dwout_hbm,
    spA_xn, spA_phq, spA_phk, spA_v, spB_xn, spB_u,
    wqkv, wo_raw, WpT, Wp, woT, wo, winT, win, woutT, wout, wsp,
    dWp, dwo_acc, dwin_acc, dwout_acc, dbsp_acc,
    xT, xnA, rstdA, phq, phk, vT, oT, dinv,
    xnB, rstdB, uT, z2n, rstd2, gT, du1, dgT,
    kv_acc, z_acc, KVT, KV, zb, dKVT, dKV, dzb,
    stA, stB,
    sems,
):
    def cp(src, dst, i):
        return pltpu.make_async_copy(src, dst, sems.at[i])

    SEM_X, SEM_G, SEM_WQKV, SEM_WO, SEM_WIN, SEM_WSP, SEM_WOUT = range(7)
    SEM_SP = 7
    SEM_OUT = 13
    SEM_GX = SEM_OUT + NT
    SEM_DW = SEM_GX + NT
    SEM_DWSP = SEM_DW + 4

    in_copies = [
        cp(x_hbm, stA, SEM_X),
        cp(wqkv_hbm, wqkv, SEM_WQKV),
        cp(wo_hbm, wo_raw, SEM_WO),
        cp(win_hbm, win, SEM_WIN),
        cp(wout_hbm, wout, SEM_WOUT),
        cp(wsp_hbm, wsp, SEM_WSP),
        cp(gout_hbm, stB, SEM_G),
    ]
    for c in in_copies:
        c.start()

    spill_pairs = [(xnA, spA_xn), (phq, spA_phq), (phk, spA_phk), (vT, spA_v),
                   (xnB, spB_xn), (uT, spB_u)]

    def spill(i):
        return cp(spill_pairs[i][0], spill_pairs[i][1], SEM_SP + i)

    def reload(i):
        return cp(spill_pairs[i][1], spill_pairs[i][0], SEM_SP + i)

    def tsl(j):
        return pl.ds(pl.multiple_of(j * T, T), T)

    dWp[...] = jnp.zeros(dWp.shape, f32)
    dwo_acc[...] = jnp.zeros(dwo_acc.shape, f32)
    dwin_acc[...] = jnp.zeros(dwin_acc.shape, f32)
    dwout_acc[...] = jnp.zeros(dwout_acc.shape, f32)
    dbsp_acc[...] = jnp.zeros(dbsp_acc.shape, f32)

    def head_mask_T():
        r = _iota((D, D), 0)
        c = _iota((D, D), 1)
        return (c // DH) == ((r // GV) * HG + (r % HG))

    def perm_T():
        r = _iota((D, D), 0)
        c = _iota((D, D), 1)
        same_head = (c // DH) == ((r // GV) * HG + (r % HG))
        same_feat = (c % DH) == ((r % GV) // HG)
        return jnp.where(same_head & same_feat, 1.0, 0.0).astype(bf16)

    def phi_T():
        e = jnp.where((_iota((128, D), 1) % DH) == _iota((128, D), 0), 1.0, 0.0).astype(bf16)
        full = _nn(wphi_ref[...], e)
        return jnp.where(head_mask_T(), full, 0.0).astype(bf16)

    eye128 = _eye(128)

    in_copies[1].wait()
    PT = phi_T()
    PiT = perm_T()
    for i in range(3):
        L = PiT if i == 2 else PT
        w = wqkv[:, i * D:(i + 1) * D]
        WpT[i * D:(i + 1) * D, :] = _nt(L, w).astype(bf16)
        Wp[:, i * D:(i + 1) * D] = _nt(w, L).astype(bf16)
    in_copies[2].wait()
    wo_p = _nn(PiT, wo_raw[...]).astype(bf16)
    wo[...] = wo_p
    for b in range(D // 128):
        woT[b * 128:(b + 1) * 128, :] = _nt(eye128, wo_p[:, b * 128:(b + 1) * 128]).astype(bf16)
    in_copies[3].wait()
    for b in range(F // 128):
        winT[b * 128:(b + 1) * 128, :] = _nt(eye128, win[:, b * 128:(b + 1) * 128]).astype(bf16)
    in_copies[4].wait()
    for b in range(D // 128):
        woutT[b * 128:(b + 1) * 128, :] = _nt(eye128, wout[:, b * 128:(b + 1) * 128]).astype(bf16)

    def load_T(st, j):
        rows = tsl(j)
        for b in range(D // 128):
            xT[b * 128:(b + 1) * 128, tsl(j)] = _nt(eye128, st[rows, b * 128:(b + 1) * 128])

    def store_T(val, st, j):
        vb = val.astype(bf16)
        for b in range(NL):
            r0 = pl.multiple_of(j * T + b * 128, 128)
            st[pl.ds(r0, 128), :] = _nt(eye128, vb[:, b * 128:(b + 1) * 128]).astype(bf16)

    in_copies[0].wait()

    def _ld(j, c):
        load_T(stA, j)
        return c

    lax.fori_loop(0, NT, _ld, 0)

    def fa1(j):
        sl = tsl(j)
        xn, rstd = _ln_fwd(xT[:, sl])
        xb = xn.astype(bf16)
        xnA[:, sl] = xb
        rstdA[:, sl] = rstd
        qkv = _nn(WpT[...], xb)
        pq_ = _phi_fwd(qkv[0:D])
        phq[:, sl] = pq_.astype(bf16)
        pk_ = _phi_fwd(qkv[D:2 * D]).astype(bf16)
        phk[:, sl] = pk_
        vb = qkv[2 * D:3 * D].astype(bf16)
        vT[:, sl] = vb
        for g in range(NG):
            kv_acc[g] += _nt(vb[g * GV:(g + 1) * GV], pk_[g * GP:(g + 1) * GP])
        z_acc[...] += _fold(pk_.astype(f32))

    def grp_mask():
        return (_iota((GV, GP), 0) % HG) == (_iota((GV, GP), 1) % HG)

    def finalize(dst_T, dst, dst_z):
        m = grp_mask()
        eye = _eye(GP)
        for g in range(NG):
            kt = jnp.where(m, kv_acc[g], 0.0).astype(bf16)
            dst_T[g] = kt
            dst[g] = _nt(eye, kt).astype(bf16)
        zs = jnp.sum(z_acc[...], axis=1, keepdims=True)
        dst_z[...] = jnp.broadcast_to(zs, (2 * D, 128))

    def zero_attn_acc():
        kv_acc[...] = jnp.zeros(kv_acc.shape, f32)
        z_acc[...] = jnp.zeros(z_acc.shape, f32)

    def fa2(j, l):
        sl = tsl(j)
        pb = phq[:, sl]
        num = jnp.concatenate(
            [_nn(KVT[l, g], pb[g * GP:(g + 1) * GP]) for g in range(NG)], axis=0)
        zt = _tile_lanes(zb[l])
        den = jnp.sum((pb.astype(f32) * zt).reshape(NG, 2 * DH, HG, T), axis=1) + 1e-6
        di = 1.0 / den
        dinv[l, :, sl] = di.reshape(H, T)
        o = (num.reshape(NG, DH, HG, T) * di[:, None]).reshape(D, T).astype(bf16)
        oT[l, :, sl] = o
        xT[:, sl] = xT[:, sl] + _nn(woT[...], o)

    def fb1(j, l):
        sl = tsl(j)
        xn, rstd = _ln_fwd(xT[:, sl])
        xb = xn.astype(bf16)
        xnB[:, sl] = xb
        rstdB[:, sl] = rstd
        u = _nn(winT[...], xb)
        uT[:, sl] = u.astype(bf16)
        z2 = _gelu(u[FH:])
        zn, r2 = _ln_fwd(z2)
        z2n[l, :, sl] = zn.astype(bf16)
        rstd2[l, :, sl] = r2

    def fb2(j, l):
        sl = tsl(j)
        g = _nt(z2n[l], wsp[sl, :]) + bsp_ref[:, sl].astype(f32)
        z1 = _gelu(uT[0:FH, sl].astype(f32))
        h = (z1 * g).astype(bf16)
        xT[:, sl] = xT[:, sl] + _nn(woutT[...], h)
        return g

    def bb1(j, l, g):
        sl = tsl(j)
        dy = xT[:, sl].astype(bf16)
        dh = _nn(wout[...], dy)
        z1, dgel = _gelu_and_grad(uT[0:FH, sl].astype(f32))
        h = (z1 * g).astype(bf16)
        dwout_acc[...] += _nt(h, dy)
        dg = dh * z1
        dbsp_acc[:, sl] += jnp.sum(dg, axis=0, keepdims=True)
        dgT[l, :, sl] = dg.astype(bf16)
        du1[:, sl] = (dh * g * dgel).astype(bf16)

    def bb2(j, l):
        sl = tsl(j)
        dzn = _nn(dgT[l], wsp[:, sl])
        dz2 = _ln_bwd(dzn, z2n[l, :, sl].astype(f32), rstd2[l, :, sl])
        du2 = (dz2 * _gelu_grad(uT[FH:, sl].astype(f32))).astype(bf16)
        du = jnp.concatenate([du1[:, sl], du2], axis=0)
        dxn = _nn(win[...], du)
        xb = xnB[:, sl]
        dwin_acc[...] += _nt(xb, du)
        xT[:, sl] = xT[:, sl] + _ln_bwd(dxn, xb.astype(f32), rstdB[:, sl])

    def ba1(j, l):
        sl = tsl(j)
        dy = xT[:, sl].astype(bf16)
        do = _nn(wo[...], dy)
        ob = oT[l, :, sl]
        dwo_acc[...] += _nt(ob, dy)
        di = dinv[l, :, sl].reshape(NG, HG, T)
        do4 = do.reshape(NG, DH, HG, T)
        dnum = (do4 * di[:, None]).reshape(D, T).astype(bf16)
        dden = -jnp.sum(do4 * ob.astype(f32).reshape(NG, DH, HG, T), axis=1) * di
        pb = phq[:, sl]
        pf = pb.astype(f32)
        dph = jnp.concatenate(
            [_nn(KV[l, g], dnum[g * GV:(g + 1) * GV]) for g in range(NG)], axis=0)
        zt = _tile_lanes(zb[l]).reshape(NG, 2 * DH, HG, T)
        dph = (dph.reshape(NG, 2 * DH, HG, T) + dden[:, None] * zt).reshape(2 * D, T)
        for g in range(NG):
            kv_acc[g] += _nt(dnum[g * GV:(g + 1) * GV], pb[g * GP:(g + 1) * GP])
        z_acc[...] += _fold((pf.reshape(NG, 2 * DH, HG, T) * dden[:, None]).reshape(2 * D, T))
        oT[l, :, sl] = _phi_bwd(pf, dph).astype(bf16)

    def ba2(j, l):
        sl = tsl(j)
        vb = vT[:, sl]
        kb = phk[:, sl]
        dph = jnp.concatenate(
            [_nn(dKV[g], vb[g * GV:(g + 1) * GV]) for g in range(NG)], axis=0)
        dph = dph + _tile_lanes(dzb[...])
        dv = jnp.concatenate(
            [_nn(dKVT[g], kb[g * GP:(g + 1) * GP]) for g in range(NG)], axis=0)
        dpk = _phi_bwd(kb.astype(f32), dph)
        dqkv = jnp.concatenate([oT[l, :, sl], dpk.astype(bf16), dv.astype(bf16)], axis=0)
        dxn = _nn(Wp[...], dqkv)
        xb = xnA[:, sl]
        dWp[...] += _nt(xb, dqkv)
        xT[:, sl] = xT[:, sl] + _ln_bwd(dxn, xb.astype(f32), rstdA[l, :, sl])

    def loop(fn):
        def body(j, c):
            fn(j)
            return c
        lax.fori_loop(0, NT, body, 0)

    class _RstdA:
        pass

    rstdA_full = rstdA

    def run_fa1(l):
        def fn(j):
            sl = tsl(j)
            xn, rstd = _ln_fwd(xT[:, sl])
            xb = xn.astype(bf16)
            xnA[:, sl] = xb
            rstdA_full[l, :, sl] = rstd
            qkv = _nn(WpT[...], xb)
            phq[:, sl] = _phi_fwd(qkv[0:D]).astype(bf16)
            pk_ = _phi_fwd(qkv[D:2 * D]).astype(bf16)
            phk[:, sl] = pk_
            vb = qkv[2 * D:3 * D].astype(bf16)
            vT[:, sl] = vb
            for g in range(NG):
                kv_acc[g] += _nt(vb[g * GV:(g + 1) * GV], pk_[g * GP:(g + 1) * GP])
            z_acc[...] += _fold(pk_.astype(f32))
        return fn

    rstdB_full = rstdB

    def run_fb1(l):
        def fn(j):
            sl = tsl(j)
            xn, rstd = _ln_fwd(xT[:, sl])
            xb = xn.astype(bf16)
            xnB[:, sl] = xb
            rstdB_full[l, :, sl] = rstd
            u = _nn(winT[...], xb)
            uT[:, sl] = u.astype(bf16)
            z2 = _gelu(u[FH:])
            zn, r2 = _ln_fwd(z2)
            z2n[l, :, sl] = zn.astype(bf16)
            rstd2[l, :, sl] = r2
        return fn

    def run_bb2(l):
        def fn(j):
            sl = tsl(j)
            dzn = _nn(dgT[l], wsp[:, sl])
            dz2 = _ln_bwd(dzn, z2n[l, :, sl].astype(f32), rstd2[l, :, sl])
            du2 = (dz2 * _gelu_grad(uT[FH:, sl].astype(f32))).astype(bf16)
            du = jnp.concatenate([du1[:, sl], du2], axis=0)
            dxn = _nn(win[...], du)
            xb = xnB[:, sl]
            dwin_acc[...] += _nt(xb, du)
            xT[:, sl] = xT[:, sl] + _ln_bwd(dxn, xb.astype(f32), rstdB_full[l, :, sl])
        return fn

    zero_attn_acc()
    loop(run_fa1(0))
    finalize(KVT.at[0], KV.at[0], zb.at[0])
    for i in range(4):
        spill(i).start()

    fb1_0 = run_fb1(0)

    def ph2(j):
        fa2(j, 0)
        fb1_0(j)

    loop(ph2)
    for i in range(4, 6):
        spill(i).start()
    for i in range(4):
        spill(i).wait()
    in_copies[5].wait()

    zero_attn_acc()
    fa1_1 = run_fa1(1)

    def ph3(j):
        g = fb2(j, 0)
        gT[:, tsl(j)] = g.astype(bf16)
        fa1_1(j)

    loop(ph3)
    finalize(KVT.at[1], KV.at[1], zb.at[1])
    for i in range(4, 6):
        spill(i).wait()

    fb1_1 = run_fb1(1)

    def ph4(j):
        fa2(j, 1)
        fb1_1(j)

    loop(ph4)

    in_copies[6].wait()

    def ph5(j):
        g = fb2(j, 1)
        store_T(xT[:, tsl(j)], stA, j)
        cp(stA.at[tsl(j)], out_hbm.at[tsl(j)], SEM_OUT + j).start()
        load_T(stB, j)
        bb1(j, 1, g)

    loop(ph5)

    zero_attn_acc()
    bb2_1 = run_bb2(1)

    def ph6(j):
        bb2_1(j)
        ba1(j, 1)

    loop(ph6)
    finalize(dKVT, dKV, dzb)
    reload(4).start()
    reload(5).start()
    reload(1).start()

    loop(lambda j: ba2(j, 1))
    reload(4).wait()
    reload(5).wait()
    reload(1).wait()
    reload(0).start()
    reload(2).start()
    reload(3).start()

    loop(lambda j: bb1(j, 0, gT[:, tsl(j)].astype(f32)))

    zero_attn_acc()
    bb2_0 = run_bb2(0)

    def ph9(j):
        bb2_0(j)
        ba1(j, 0)

    loop(ph9)
    finalize(dKVT, dKV, dzb)
    reload(0).wait()
    reload(2).wait()
    reload(3).wait()

    def ph10(j):
        ba2(j, 0)
        store_T(xT[:, tsl(j)], stB, j)
        cp(stB.at[tsl(j)], gx_hbm.at[tsl(j)], SEM_GX + j).start()

    loop(ph10)

    PT = phi_T()
    PiT = perm_T()
    xacc = jnp.zeros((D, D), f32)
    for i in range(2):
        hi, lo = _split_hi_lo(dWp[:, i * D:(i + 1) * D])
        Wp[:, i * D:(i + 1) * D] = (_nn(hi, PT) + _nn(lo, PT)).astype(bf16)
        w = wqkv[:, i * D:(i + 1) * D]
        xacc = xacc + _tn(w, hi) + _tn(w, lo)
    Wp[:, 2 * D:3 * D] = _nn(dWp[:, 2 * D:3 * D].astype(bf16), PiT).astype(bf16)
    dw_copies = [cp(Wp, dwqkv_hbm, SEM_DW)]
    dw_copies[0].start()
    r = _iota((D, D), 0)
    c = _iota((D, D), 1)
    xm = jnp.where((r // DH) == ((c // GV) * HG + (c % HG)), xacc, 0.0)
    e2 = jnp.where(((_iota((D, 128), 0) % GV) // HG) == _iota((D, 128), 1), 1.0, 0.0).astype(bf16)
    hi, lo = _split_hi_lo(xm)
    dwphi_ref[...] = (_nn(hi, e2) + _nn(lo, e2)).astype(bf16)
    wo[...] = _tn(PiT, dwo_acc[...].astype(bf16)).astype(bf16)
    win[...] = dwin_acc[...].astype(bf16)
    wout[...] = dwout_acc[...].astype(bf16)
    dbsp_ref[...] = dbsp_acc[...].astype(bf16)
    dw_copies += [cp(wo, dwo_hbm, SEM_DW + 1), cp(win, dwin_hbm, SEM_DW + 2),
                  cp(wout, dwout_hbm, SEM_DW + 3)]
    for c_ in dw_copies[1:]:
        c_.start()

    def dwsp_copy(j):
        slot = j % 2
        return cp(phq.at[slot * T:(slot + 1) * T], dwsp_hbm.at[j * T:(j + 1) * T], SEM_DWSP + slot)

    for j in range(NT):
        if j >= 2:
            dwsp_copy(j - 2).wait()
        acc = None
        for l in range(2):
            dgn = jnp.concatenate(
                [_nt(eye128, dgT[l, :, j * T + b * 128: j * T + (b + 1) * 128]).astype(bf16)
                 for b in range(NL)], axis=0)
            t = _nn(dgn, z2n[l])
            acc = t if acc is None else acc + t
        slot = j % 2
        phq[slot * T:(slot + 1) * T, :] = acc.astype(bf16)
        dwsp_copy(j).start()

    for j in range(max(NT - 2, 0), NT):
        dwsp_copy(j).wait()
    for c_ in dw_copies:
        c_.wait()
    for j in range(NT):
        cp(stA.at[j * T:(j + 1) * T], out_hbm.at[j * T:(j + 1) * T], SEM_OUT + j).wait()
        cp(stB.at[j * T:(j + 1) * T], gx_hbm.at[j * T:(j + 1) * T], SEM_GX + j).wait()


@jax.jit
def pallas_interleave_layers__linear_kernel_hedgehog__mixer_gmlp__prompt_kernel(
    A_x: jax.Array,
    A_wqkv: jax.Array,
    A_w_phi: jax.Array,
    A_wo: jax.Array,
    B_x: jax.Array,
    B_w_in: jax.Array,
    B_w_sp: jax.Array,
    B_b_sp: jax.Array,
    B_w_out: jax.Array,
    grad_out: jax.Array,
):
    del B_x
    x = A_x.reshape(S, D)
    gout = grad_out.reshape(S, D)
    wphi_t = A_w_phi.reshape(NG, HG, DH, DH).transpose(0, 3, 1, 2).reshape(D, DH)
    wphi_t = jnp.pad(wphi_t, ((0, 0), (0, 128 - DH)))
    bsp = B_b_sp.reshape(1, S)

    any_spec = pl.BlockSpec(memory_space=pl.ANY)
    vmem_spec = pl.BlockSpec(memory_space=pltpu.VMEM)

    out_shape = (
        jax.ShapeDtypeStruct((S, D), bf16),
        jax.ShapeDtypeStruct((S, D), bf16),
        jax.ShapeDtypeStruct((D, 3 * D), bf16),
        jax.ShapeDtypeStruct((D, 128), bf16),
        jax.ShapeDtypeStruct((D, D), bf16),
        jax.ShapeDtypeStruct((D, F), bf16),
        jax.ShapeDtypeStruct((S, S), bf16),
        jax.ShapeDtypeStruct((1, S), bf16),
        jax.ShapeDtypeStruct((FH, D), bf16),
        jax.ShapeDtypeStruct((D, S), bf16),
        jax.ShapeDtypeStruct((2 * D, S), bf16),
        jax.ShapeDtypeStruct((2 * D, S), bf16),
        jax.ShapeDtypeStruct((D, S), bf16),
        jax.ShapeDtypeStruct((D, S), bf16),
        jax.ShapeDtypeStruct((F, S), bf16),
    )
    out_specs = (any_spec, any_spec, any_spec, vmem_spec, any_spec, any_spec, any_spec,
                 vmem_spec, any_spec) + (any_spec,) * 6
    in_specs = [any_spec, any_spec, any_spec, vmem_spec, any_spec, any_spec, any_spec,
                vmem_spec, any_spec]

    V = pltpu.VMEM
    scratch = [
        V((D, 3 * D), bf16), V((D, D), bf16), V((3 * D, D), bf16), V((D, 3 * D), bf16),
        V((D, D), bf16), V((D, D), bf16), V((F, D), bf16), V((D, F), bf16),
        V((D, FH), bf16), V((FH, D), bf16), V((S, S), bf16),
        V((D, 3 * D), f32), V((D, D), f32), V((D, F), f32), V((FH, D), f32), V((1, S), f32),
        V((D, S), f32), V((D, S), bf16), V((2, 1, S), f32), V((2 * D, S), bf16),
        V((2 * D, S), bf16), V((D, S), bf16), V((2, D, S), bf16), V((2, H, S), f32),
        V((D, S), bf16), V((2, 1, S), f32), V((F, S), bf16), V((2, FH, S), bf16),
        V((2, 1, S), f32), V((FH, S), bf16), V((FH, S), bf16), V((2, FH, S), bf16),
        V((NG, GV, GP), f32), V((2 * D, 128), f32),
        V((2, NG, GV, GP), bf16), V((2, NG, GP, GV), bf16), V((2, 2 * D, 128), f32),
        V((NG, GV, GP), bf16), V((NG, GP, GV), bf16), V((2 * D, 128), f32),
        V((S, D), bf16), V((S, D), bf16),
        pltpu.SemaphoreType.DMA((13 + 2 * NT + 4 + 2,)),
    ]

    res = pl.pallas_call(
        _kernel,
        out_shape=out_shape,
        in_specs=in_specs,
        out_specs=out_specs,
        scratch_shapes=scratch,
        compiler_params=pltpu.CompilerParams(vmem_limit_bytes=126 * 1024 * 1024),
    )(x, gout, A_wqkv, wphi_t, A_wo, B_w_in, B_w_sp, bsp, B_w_out)

    out, gx, dwqkv, dwphi, dwo, dwin, dwsp, dbsp, dwout = res[:9]
    return (
        out.reshape(1, S, D),
        gx.reshape(1, S, D),
        dwqkv,
        dwphi[:, :DH].reshape(H, DH, DH),
        dwo,
        dwin,
        dwsp,
        dbsp.reshape(S),
        dwout,
    )
```

```python
import jax
import jax.numpy as jnp
from jax import lax
import jax.experimental.pallas as pl
import jax.experimental.pallas.tpu as pltpu

S = 2048
D = 640
H = 32
DH = 20
NG = 8
HG = 4
GV = DH * HG
GP = 2 * GV
DP = DH // 2
F = 1536
FH = 768
T = 512
NT = S // T
TS = 256
NL = T // 128
EPS = 1e-5
GELU_C = 0.7978845608028654
GELU_A = 0.044715

f32 = jnp.float32
bf16 = jnp.bfloat16

_NT = (((1,), (1,)), ((), ()))
_TN = (((0,), (0,)), ((), ()))


def _nn(a, b):
    return jnp.dot(a, b, preferred_element_type=f32)


def _nt(a, b):
    return lax.dot_general(a, b, _NT, preferred_element_type=f32)


def _tn(a, b):
    return lax.dot_general(a, b, _TN, preferred_element_type=f32)


def _iota(shape, dim):
    return lax.broadcasted_iota(jnp.int32, shape, dim)


def _ln_fwd(x):
    mu = jnp.mean(x, axis=0, keepdims=True)
    xc = x - mu
    var = jnp.mean(xc * xc, axis=0, keepdims=True)
    rstd = lax.rsqrt(var + EPS)
    return xc * rstd, rstd


def _ln_bwd(dxn, xn, rstd):
    m1 = jnp.mean(dxn, axis=0, keepdims=True)
    m2 = jnp.mean(dxn * xn, axis=0, keepdims=True)
    return rstd * (dxn - m1 - xn * m2)


def _gelu(u):
    t = jnp.tanh(GELU_C * (u + GELU_A * (u * u * u)))
    return 0.5 * u * (1.0 + t)


def _gelu_and_grad(u):
    u2 = u * u
    t = jnp.tanh(GELU_C * (u + GELU_A * (u2 * u)))
    hp = 0.5 * (1.0 + t)
    g = u * hp
    dg = hp + (0.5 * GELU_C) * u * (1.0 - t * t) * (1.0 + (3.0 * GELU_A) * u2)
    return g, dg


def _gelu_grad(u):
    return _gelu_and_grad(u)[1]


def _half_sum(a):
    return a + pltpu.roll(a, 4, 1)


def _phi_fwd(p):
    p4 = p.reshape(NG, DP, 8, T)
    mx = jnp.max(p4, axis=1)
    mn = jnp.min(p4, axis=1)
    mx = jnp.maximum(mx, pltpu.roll(mx, 4, 1))[:, None]
    mn = jnp.minimum(mn, pltpu.roll(mn, 4, 1))[:, None]
    ep = jnp.exp(p4 - mx)
    em = jnp.exp(mn - p4)
    rp = 1.0 / _half_sum(jnp.sum(ep, axis=1))
    rm = 1.0 / _half_sum(jnp.sum(em, axis=1))
    ph = jnp.concatenate([ep * rp[:, None], em * rm[:, None]], axis=1)
    return ph.reshape(2 * D, T)


def _phi_bwd(ph, dph):
    ph4 = ph.reshape(NG, 2 * DP, 8, T)
    dph4 = dph.reshape(NG, 2 * DP, 8, T)
    php, phm = ph4[:, :DP], ph4[:, DP:]
    tp = php * dph4[:, :DP]
    tm = phm * dph4[:, DP:]
    sp = _half_sum(jnp.sum(tp, axis=1))[:, None]
    sm = _half_sum(jnp.sum(tm, axis=1))[:, None]
    dp = (tp - php * sp) - (tm - phm * sm)
    return dp.reshape(D, T)


def _fold(a):
    r = a[:, 0:128]
    for i in range(1, NL):
        r = r + a[:, i * 128:(i + 1) * 128]
    return r


def _tile_lanes(a):
    return jnp.concatenate([a] * NL, axis=1)


def _split_hi_lo(a):
    hi = a.astype(bf16)
    lo = (a - hi.astype(f32)).astype(bf16)
    return hi, lo


def _kernel(
    x_hbm, gout_hbm, wqkv_hbm, wphi_ref, wo_hbm, win_hbm, wsp_hbm, bsp_ref, wout_hbm,
    out_hbm, gx_hbm, dwqkv_hbm, dwphi_ref, dwo_hbm, dwin_hbm, dwsp_hbm, dbsp_ref, dwout_hbm,
    spA_xn, spA_phq, spA_phk, spA_v, spB_xn, spB_u,
    wqkv, wo_raw, WpT, Wp, woT, wo, winT, win, woutT, wout, wsp,
    dWp, dwo_acc, dwin_acc, dwout_acc, dbsp_acc,
    xT, xnA, rstdA, phq, phk, vT, oT, dinv,
    xnB, rstdB, uT, z2n, rstd2, gT, du1, dgT,
    kv_acc, z_acc, KVT, KV, zb, dKVT, dKV, dzb,
    stA, stB,
    sems,
):
    def cp(src, dst, i):
        return pltpu.make_async_copy(src, dst, sems.at[i])

    SEM_X, SEM_G, SEM_WQKV, SEM_WO, SEM_WIN, SEM_WSP, SEM_WOUT = range(7)
    SEM_SP = 7
    SEM_OUT = 13
    SEM_XT = 13 + 2 * NT + 4 + 2
    SEM_W3 = SEM_XT + NT
    SEM_GX = SEM_OUT + NT
    SEM_DW = SEM_GX + NT
    SEM_DWSP = SEM_DW + 4

    in_copies = [
        None,
        None,
        cp(wo_hbm, wo_raw, SEM_WO),
        cp(win_hbm, win, SEM_WIN),
        cp(wout_hbm, wout, SEM_WOUT),
        cp(wsp_hbm, wsp, SEM_WSP),
        cp(gout_hbm, stB, SEM_G),
    ]
    def w3_copy(i):
        return cp(wqkv_hbm.at[:, i * D:(i + 1) * D], wqkv.at[:, i * D:(i + 1) * D], SEM_W3 + i)

    def xt_copy(j):
        rows = pl.ds(pl.multiple_of(j * T, T), T)
        return cp(x_hbm.at[rows], stA.at[rows], SEM_XT + j)

    for i in range(3):
        w3_copy(i).start()
    for j in range(NT):
        xt_copy(j).start()

    spill_pairs = [(xnA, spA_xn), (phq, spA_phq), (phk, spA_phk), (vT, spA_v),
                   (xnB, spB_xn), (uT, spB_u)]

    def spill(i):
        return cp(spill_pairs[i][0], spill_pairs[i][1], SEM_SP + i)

    def reload(i):
        return cp(spill_pairs[i][1], spill_pairs[i][0], SEM_SP + i)

    def tsl(j):
        return pl.ds(pl.multiple_of(j * T, T), T)

    dWp[...] = jnp.zeros(dWp.shape, f32)
    dwo_acc[...] = jnp.zeros(dwo_acc.shape, f32)
    dwin_acc[...] = jnp.zeros(dwin_acc.shape, f32)
    dwout_acc[...] = jnp.zeros(dwout_acc.shape, f32)
    dbsp_acc[...] = jnp.zeros(dbsp_acc.shape, f32)

    def row_ids(fn):
        r = fn(_iota((D, 128), 0))
        return jnp.concatenate([r] * (D // 128), axis=1)

    def col_ids(fn, rows=D):
        c = fn(_iota((8, D), 1))
        return jnp.broadcast_to(c[0:1], (rows, D))

    def grp_head(i):
        return (i // GV) * HG + (i % HG)

    def grp_feat(i):
        return (i % GV) // HG

    def head_mask_T():
        return col_ids(lambda c: c // DH) == row_ids(grp_head)

    def perm_T():
        same_feat = col_ids(lambda c: c % DH) == row_ids(grp_feat)
        return jnp.where(head_mask_T() & same_feat, 1.0, 0.0).astype(bf16)

    def phi_T():
        e = jnp.where(col_ids(lambda c: c % DH, 128) == _iota((128, D), 0), 1.0, 0.0).astype(bf16)
        full = _nn(wphi_ref[...], e)
        return jnp.where(head_mask_T(), full, 0.0).astype(bf16)

    NB = D // 128

    def tri(b):
        return max(b - 1, 0) * 128, min(b + 2, NB) * 128

    PT = phi_T()
    PiT = perm_T()
    for i in range(3):
        L = PiT if i == 2 else PT
        w3_copy(i).wait()
        if i == 2:
            for c in in_copies[2:]:
                c.start()
        for b in range(NB):
            k0, k1 = tri(b)
            blk = _nt(wqkv[:, i * D + k0:i * D + k1], L[b * 128:(b + 1) * 128, k0:k1])
            Wp[:, i * D + b * 128:i * D + (b + 1) * 128] = blk.astype(bf16)
            WpT[i * D + b * 128:i * D + (b + 1) * 128, :] = blk.T.astype(bf16)

    def setup_rest():
        PiT_ = perm_T()
        in_copies[2].wait()
        for b in range(NB):
            k0, k1 = tri(b)
            blk = _nn(PiT_[b * 128:(b + 1) * 128, k0:k1], wo_raw[k0:k1, :])
            wo[b * 128:(b + 1) * 128, :] = blk.astype(bf16)
            woT[:, b * 128:(b + 1) * 128] = blk.T.astype(bf16)
        in_copies[3].wait()
        for b in range(F // 512):
            winT[b * 512:(b + 1) * 512, :] = win[:, b * 512:(b + 1) * 512].astype(f32).T.astype(bf16)
        in_copies[4].wait()
        woutT[...] = wout[...].astype(f32).T.astype(bf16)

    def load_T(st, j):
        xT[:, tsl(j)] = st[tsl(j), :].astype(f32).T

    def store_T(val, st, j):
        st[tsl(j), :] = val.T.astype(bf16)


    def grp_mask():
        return (_iota((GV, GP), 0) % HG) == (_iota((GV, GP), 1) % HG)

    def finalize(dst_T, dst, dst_z):
        m = grp_mask()
        for g in range(NG):
            kt = jnp.where(m, kv_acc[g], 0.0)
            dst_T[g] = kt.astype(bf16)
            dst[g] = kt.T.astype(bf16)
        zs = jnp.sum(z_acc[...], axis=1, keepdims=True)
        dst_z[...] = jnp.broadcast_to(zs, (2 * D, 128))

    def zero_attn_acc():
        kv_acc[...] = jnp.zeros(kv_acc.shape, f32)
        z_acc[...] = jnp.zeros(z_acc.shape, f32)

    def fa1(j, l):
        sl = tsl(j)
        xn, rstd = _ln_fwd(xT[:, sl])
        xb = xn.astype(bf16)
        xnA[:, sl] = xb
        rstdA[l, :, sl] = rstd
        pk = _nn(WpT[D:2 * D, :], xb)
        vb = _nn(WpT[2 * D:3 * D, :], xb).astype(bf16)
        vT[:, sl] = vb
        pk_ = _phi_fwd(pk).astype(bf16)
        phk[:, sl] = pk_
        pq = _nn(WpT[0:D, :], xb)
        for g in range(NG):
            kv_acc[g] += _nt(vb[g * GV:(g + 1) * GV], pk_[g * GP:(g + 1) * GP])
        phq[:, sl] = _phi_fwd(pq).astype(bf16)
        z_acc[...] += _fold(pk_.astype(f32))

    def fa2(j, l):
        sl = tsl(j)
        pb = phq[:, sl]
        num = jnp.concatenate(
            [_nn(KVT[l, g], pb[g * GP:(g + 1) * GP]) for g in range(NG)], axis=0)
        zt = _tile_lanes(zb[l])
        den = _half_sum(jnp.sum((pb.astype(f32) * zt).reshape(NG, 2 * DP, 8, T), axis=1)) + 1e-6
        di = 1.0 / den
        dinv[l, :, sl] = di.reshape(NG * 8, T)
        o = (num.reshape(NG, DP, 8, T) * di[:, None]).reshape(D, T).astype(bf16)
        oT[l, :, sl] = o
        xT[:, sl] = xT[:, sl] + _nn(woT[...], o)

    def fb1(j, l):
        sl = tsl(j)
        xn, rstd = _ln_fwd(xT[:, sl])
        xb = xn.astype(bf16)
        xnB[:, sl] = xb
        rstdB[l, :, sl] = rstd
        u2 = _nn(winT[FH:, :], xb)
        uT[0:FH, sl] = _nn(winT[0:FH, :], xb).astype(bf16)
        uT[FH:, sl] = u2.astype(bf16)
        zn, r2 = _ln_fwd(_gelu(u2))
        z2n[l, :, sl] = zn.astype(bf16)
        rstd2[l, :, sl] = r2

    def fb2(j, l):
        sl = tsl(j)
        g = _nt(z2n[l], wsp[sl, :]) + bsp_ref[:, sl].astype(f32)
        z1 = _gelu(uT[0:FH, sl].astype(f32))
        h = (z1 * g).astype(bf16)
        xT[:, sl] = xT[:, sl] + _nn(woutT[...], h)
        return g

    def bb1(j, l, g):
        sl = tsl(j)
        dy = xT[:, sl].astype(bf16)
        dh = _nn(wout[...], dy)
        z1, dgel = _gelu_and_grad(uT[0:FH, sl].astype(f32))
        h = (z1 * g).astype(bf16)
        dwout_acc[...] += _nt(h, dy)
        dg = dh * z1
        dbsp_acc[:, sl] += jnp.sum(dg, axis=0, keepdims=True)
        dgT[l, :, sl] = dg.astype(bf16)
        du1[:, sl] = (dh * g * dgel).astype(bf16)

    def bb2(j, l):
        sl = tsl(j)
        dzn = _nn(dgT[l], wsp[:, sl])
        gg = _gelu_grad(uT[FH:, sl].astype(f32))
        xb = xnB[:, sl]
        d1 = du1[:, sl]
        dxn1 = _nn(win[:, 0:FH], d1)
        dwin_acc[:, 0:FH] += _nt(xb, d1)
        dz2 = _ln_bwd(dzn, z2n[l, :, sl].astype(f32), rstd2[l, :, sl])
        du2 = (dz2 * gg).astype(bf16)
        dxn = dxn1 + _nn(win[:, FH:], du2)
        dwin_acc[:, FH:] += _nt(xb, du2)
        xT[:, sl] = xT[:, sl] + _ln_bwd(dxn, xb.astype(f32), rstdB[l, :, sl])

    def ba1(j, l):
        sl = tsl(j)
        dy = xT[:, sl].astype(bf16)
        do = _nn(wo[...], dy)
        ob = oT[l, :, sl]
        dwo_acc[...] += _nt(ob, dy)
        di = dinv[l, :, sl].reshape(NG, 8, T)
        do4 = do.reshape(NG, DP, 8, T)
        dnum = (do4 * di[:, None]).reshape(D, T).astype(bf16)
        dden = -_half_sum(jnp.sum(do4 * ob.astype(f32).reshape(NG, DP, 8, T), axis=1)) * di
        pb = phq[:, sl]
        pf = pb.astype(f32)
        dph = jnp.concatenate(
            [_nn(KV[l, g], dnum[g * GV:(g + 1) * GV]) for g in range(NG)], axis=0)
        for g in range(NG):
            kv_acc[g] += _nt(dnum[g * GV:(g + 1) * GV], pb[g * GP:(g + 1) * GP])
        zt = _tile_lanes(zb[l]).reshape(NG, 2 * DP, 8, T)
        dph = (dph.reshape(NG, 2 * DP, 8, T) + dden[:, None] * zt).reshape(2 * D, T)
        z_acc[...] += _fold((pf.reshape(NG, 2 * DP, 8, T) * dden[:, None]).reshape(2 * D, T))
        oT[l, :, sl] = _phi_bwd(pf, dph).astype(bf16)

    def ba2(j, l):
        sl = tsl(j)
        vb = vT[:, sl]
        kb = phk[:, sl]
        xb = xnA[:, sl]
        dph = jnp.concatenate(
            [_nn(dKV[g], vb[g * GV:(g + 1) * GV]) for g in range(NG)], axis=0)
        dv = jnp.concatenate(
            [_nn(dKVT[g], kb[g * GP:(g + 1) * GP]) for g in range(NG)], axis=0).astype(bf16)
        dq = oT[l, :, sl]
        dxn = _nn(Wp[:, 0:D], dq)
        dWp[:, 0:D] += _nt(xb, dq)
        dpk = _phi_bwd(kb.astype(f32), dph + _tile_lanes(dzb[...])).astype(bf16)
        dxn = dxn + _nn(Wp[:, 2 * D:3 * D], dv)
        dxn = dxn + _nn(Wp[:, D:2 * D], dpk)
        dWp[:, 2 * D:3 * D] += _nt(xb, dv)
        dWp[:, D:2 * D] += _nt(xb, dpk)
        xT[:, sl] = xT[:, sl] + _ln_bwd(dxn, xb.astype(f32), rstdA[l, :, sl])

    def loop(fn):
        def body(j, c):
            fn(j)
            return c
        lax.fori_loop(0, NT, body, 0)

    def run_fa1(l):
        return lambda j: fa1(j, l)

    def run_fb1(l):
        return lambda j: fb1(j, l)

    def run_bb2(l):
        return lambda j: bb2(j, l)

    zero_attn_acc()
    def ph1(j):
        xt_copy(j).wait()
        load_T(stA, j)
        fa1(j, 0)

    loop(ph1)
    finalize(KVT.at[0], KV.at[0], zb.at[0])
    for i in range(4):
        spill(i).start()
    setup_rest()

    fb1_0 = run_fb1(0)

    def ph2(j):
        fa2(j, 0)
        fb1_0(j)

    loop(ph2)
    for i in range(4, 6):
        spill(i).start()
    for i in range(4):
        spill(i).wait()
    in_copies[5].wait()

    zero_attn_acc()
    fa1_1 = run_fa1(1)

    def ph3(j):
        g = fb2(j, 0)
        gT[:, tsl(j)] = g.astype(bf16)
        fa1_1(j)

    loop(ph3)
    finalize(KVT.at[1], KV.at[1], zb.at[1])
    for i in range(4, 6):
        spill(i).wait()

    fb1_1 = run_fb1(1)

    def ph4(j):
        fa2(j, 1)
        fb1_1(j)

    loop(ph4)

    in_copies[6].wait()

    def ph5(j):
        g = fb2(j, 1)
        store_T(xT[:, tsl(j)], stA, j)
        cp(stA.at[tsl(j)], out_hbm.at[tsl(j)], SEM_OUT + j).start()
        load_T(stB, j)
        bb1(j, 1, g)

    loop(ph5)

    zero_attn_acc()
    bb2_1 = run_bb2(1)

    def ph6(j):
        bb2_1(j)
        ba1(j, 1)

    loop(ph6)
    finalize(dKVT, dKV, dzb)
    reload(4).start()
    reload(5).start()
    reload(1).start()

    loop(lambda j: ba2(j, 1))
    reload(4).wait()
    reload(5).wait()
    reload(1).wait()
    reload(0).start()
    reload(2).start()
    reload(3).start()

    loop(lambda j: bb1(j, 0, gT[:, tsl(j)].astype(f32)))

    zero_attn_acc()
    bb2_0 = run_bb2(0)

    def ph9(j):
        bb2_0(j)
        ba1(j, 0)

    loop(ph9)
    finalize(dKVT, dKV, dzb)
    reload(0).wait()
    reload(2).wait()
    reload(3).wait()

    def ph10(j):
        ba2(j, 0)
        store_T(xT[:, tsl(j)], stB, j)
        cp(stB.at[tsl(j)], gx_hbm.at[tsl(j)], SEM_GX + j).start()

    loop(ph10)

    PT = phi_T()
    PiT = perm_T()
    xcols = []
    for b in range(NB):
        k0, k1 = tri(b)
        xb_ = None
        for i in range(2):
            t = _tn(wqkv[:, i * D + k0:i * D + k1],
                    dWp[:, i * D + b * 128:i * D + (b + 1) * 128].astype(bf16))
            xb_ = t if xb_ is None else xb_ + t
        parts = []
        if k0 > 0:
            parts.append(jnp.zeros((k0, 128), f32))
        parts.append(xb_)
        if k1 < D:
            parts.append(jnp.zeros((D - k1, 128), f32))
        xcols.append(jnp.concatenate(parts, axis=0))
    xacc = jnp.concatenate(xcols, axis=1)
    for i in range(3):
        L = PiT if i == 2 else PT
        for b in range(NB):
            k0, k1 = tri(b)
            Wp[:, i * D + b * 128:i * D + (b + 1) * 128] = _nn(
                dWp[:, i * D + k0:i * D + k1].astype(bf16), L[k0:k1, b * 128:(b + 1) * 128]).astype(bf16)
    dw_copies = [cp(Wp, dwqkv_hbm, SEM_DW)]
    dw_copies[0].start()
    xm = jnp.where(row_ids(lambda r: r // DH) == col_ids(grp_head), xacc, 0.0)
    e2 = jnp.where(grp_feat(_iota((D, 128), 0)) == _iota((D, 128), 1), 1.0, 0.0).astype(bf16)
    hi, lo = _split_hi_lo(xm)
    dwphi_ref[...] = (_nn(hi, e2) + _nn(lo, e2)).astype(bf16)
    for b in range(NB):
        k0, k1 = tri(b)
        wo[b * 128:(b + 1) * 128, :] = _tn(PiT[k0:k1, b * 128:(b + 1) * 128],
                                           dwo_acc[k0:k1, :].astype(bf16)).astype(bf16)
    win[...] = dwin_acc[...].astype(bf16)
    wout[...] = dwout_acc[...].astype(bf16)
    dbsp_ref[...] = dbsp_acc[...].astype(bf16)
    dw_copies += [cp(wo, dwo_hbm, SEM_DW + 1), cp(win, dwin_hbm, SEM_DW + 2),
                  cp(wout, dwout_hbm, SEM_DW + 3)]
    for c_ in dw_copies[1:]:
        c_.start()

    def dwsp_copy(j):
        slot = j % 2
        return cp(phq.at[slot * TS:(slot + 1) * TS], dwsp_hbm.at[j * TS:(j + 1) * TS], SEM_DWSP + slot)

    NS = S // TS
    for j in range(NS):
        if j >= 2:
            dwsp_copy(j - 2).wait()
        acc = None
        for l in range(2):
            t = _tn(dgT[l, :, j * TS:(j + 1) * TS], z2n[l])
            acc = t if acc is None else acc + t
        slot = j % 2
        phq[slot * TS:(slot + 1) * TS, :] = acc.astype(bf16)
        dwsp_copy(j).start()

    for j in range(max(NS - 2, 0), NS):
        dwsp_copy(j).wait()
    for c_ in dw_copies:
        c_.wait()
    for j in range(NT):
        cp(stA.at[j * T:(j + 1) * T], out_hbm.at[j * T:(j + 1) * T], SEM_OUT + j).wait()
        cp(stB.at[j * T:(j + 1) * T], gx_hbm.at[j * T:(j + 1) * T], SEM_GX + j).wait()


@jax.jit
def pallas_interleave_layers__linear_kernel_hedgehog__mixer_gmlp__prompt_kernel(
    A_x: jax.Array,
    A_wqkv: jax.Array,
    A_w_phi: jax.Array,
    A_wo: jax.Array,
    B_x: jax.Array,
    B_w_in: jax.Array,
    B_w_sp: jax.Array,
    B_b_sp: jax.Array,
    B_w_out: jax.Array,
    grad_out: jax.Array,
):
    del B_x
    x = A_x.reshape(S, D)
    gout = grad_out.reshape(S, D)
    wphi_t = A_w_phi.reshape(NG, HG, DH, DH).transpose(0, 3, 1, 2).reshape(D, DH)
    wphi_t = jnp.pad(wphi_t, ((0, 0), (0, 128 - DH)))
    bsp = B_b_sp.reshape(1, S)

    any_spec = pl.BlockSpec(memory_space=pl.ANY)
    vmem_spec = pl.BlockSpec(memory_space=pltpu.VMEM)

    out_shape = (
        jax.ShapeDtypeStruct((S, D), bf16),
        jax.ShapeDtypeStruct((S, D), bf16),
        jax.ShapeDtypeStruct((D, 3 * D), bf16),
        jax.ShapeDtypeStruct((D, 128), bf16),
        jax.ShapeDtypeStruct((D, D), bf16),
        jax.ShapeDtypeStruct((D, F), bf16),
        jax.ShapeDtypeStruct((S, S), bf16),
        jax.ShapeDtypeStruct((1, S), bf16),
        jax.ShapeDtypeStruct((FH, D), bf16),
        jax.ShapeDtypeStruct((D, S), bf16),
        jax.ShapeDtypeStruct((2 * D, S), bf16),
        jax.ShapeDtypeStruct((2 * D, S), bf16),
        jax.ShapeDtypeStruct((D, S), bf16),
        jax.ShapeDtypeStruct((D, S), bf16),
        jax.ShapeDtypeStruct((F, S), bf16),
    )
    out_specs = (any_spec, any_spec, any_spec, vmem_spec, any_spec, any_spec, any_spec,
                 vmem_spec, any_spec) + (any_spec,) * 6
    in_specs = [any_spec, any_spec, any_spec, vmem_spec, any_spec, any_spec, any_spec,
                vmem_spec, any_spec]

    V = pltpu.VMEM
    scratch = [
        V((D, 3 * D), bf16), V((D, D), bf16), V((3 * D, D), bf16), V((D, 3 * D), bf16),
        V((D, D), bf16), V((D, D), bf16), V((F, D), bf16), V((D, F), bf16),
        V((D, FH), bf16), V((FH, D), bf16), V((S, S), bf16),
        V((D, 3 * D), f32), V((D, D), f32), V((D, F), f32), V((FH, D), f32), V((1, S), f32),
        V((D, S), f32), V((D, S), bf16), V((2, 1, S), f32), V((2 * D, S), bf16),
        V((2 * D, S), bf16), V((D, S), bf16), V((2, D, S), bf16), V((2, NG * 8, S), f32),
        V((D, S), bf16), V((2, 1, S), f32), V((F, S), bf16), V((2, FH, S), bf16),
        V((2, 1, S), f32), V((FH, S), bf16), V((FH, S), bf16), V((2, FH, S), bf16),
        V((NG, GV, GP), f32), V((2 * D, 128), f32),
        V((2, NG, GV, GP), bf16), V((2, NG, GP, GV), bf16), V((2, 2 * D, 128), f32),
        V((NG, GV, GP), bf16), V((NG, GP, GV), bf16), V((2 * D, 128), f32),
        V((S, D), bf16), V((S, D), bf16),
        pltpu.SemaphoreType.DMA((13 + 2 * NT + 4 + 2 + NT + 3,)),
    ]

    res = pl.pallas_call(
        _kernel,
        out_shape=out_shape,
        in_specs=in_specs,
        out_specs=out_specs,
        scratch_shapes=scratch,
        compiler_params=pltpu.CompilerParams(vmem_limit_bytes=126 * 1024 * 1024),
    )(x, gout, A_wqkv, wphi_t, A_wo, B_w_in, B_w_sp, bsp, B_w_out)

    out, gx, dwqkv, dwphi, dwo, dwin, dwsp, dbsp, dwout = res[:9]
    return (
        out.reshape(1, S, D),
        gx.reshape(1, S, D),
        dwqkv,
        dwphi[:, :DH].reshape(H, DH, DH),
        dwo,
        dwin,
        dwsp,
        dbsp.reshape(S),
        dwout,
    )
```
